```python
import os as _os
_os.environ.setdefault("JAX_PLATFORMS", "cpu")
import jax
import jax.numpy as jnp

def _softmax(x, axis=-1):
    return jax.nn.softmax(x, axis=axis)
def _gelu(x):
    return jax.nn.gelu(x, approximate=True)
def _silu(x):
    return jax.nn.silu(x)
def _sigmoid(x):
    return jax.nn.sigmoid(x)
def _layernorm(x, axis=-1, eps=1e-5):
    m = jnp.mean(x, axis=axis, keepdims=True)
    v = jnp.var(x, axis=axis, keepdims=True)
    return (x - m) / jnp.sqrt(v + eps)
def _scatter_add(tgt, idx, src, axis=0):
    return tgt.at[idx].add(src)
def _segment_sum(src, seg, n):
    return jax.ops.segment_sum(src, seg, n)
class _Rng:
    def __init__(self, key):
        self._k = key
    def _next(self):
        self._k, sub = jax.random.split(self._k)
        return sub
    def normal(self, shape):
        return jax.random.normal(self._next(), shape, dtype=jnp.bfloat16)
    def randint(self, lo, hi, shape):
        return jax.random.randint(self._next(), shape, lo, hi, dtype=jnp.int32)
    def uniform(self, shape, lo=0.0, hi=1.0):
        return jax.random.uniform(self._next(), shape, jnp.bfloat16, lo, hi)
    def permutation(self, n):
        return jax.random.permutation(self._next(), n)


kernel_name = 'gated_mix__sliding_block_cached__swiglu_ffn__decode'

def setup_inputs():
    _rng = _Rng(jax.random.key(int.from_bytes(__import__("os").urandom(4), "little")))
    _w = (lambda a: (lambda t: t.astype(jnp.bfloat16) if jnp.issubdtype(t.dtype, jnp.floating) else t)(jnp.asarray(a)))
    def _A_setup():
        B, Sq, D = 1, 1, 512
        Hq, Hkv, Sk, Dh = 32, 32, 32768, 128
        assert Hq % Hkv == 0, (Hq, Hkv)
        return {
            "x": _w((lambda *s: _rng.normal(s) * 0.05)(B, Sq, D)),
            "k_cache": _w((lambda *s: _rng.normal(s) * 3.2)(B, Hkv, Sk, Dh)),
            "v_cache": _w((lambda *s: _rng.normal(s) * 1.6)(B, Hkv, Sk, Dh)),
            "wq": _w((lambda *s: _rng.normal(s) * 3.2)(D, Hq * Dh) * (D ** -0.5)),
            "wo": _w((lambda *s: _rng.normal(s) * 1.6)(Hq * Dh, D) * ((Hq * Dh) ** -0.5)),
        }
    _A_in = _A_setup()

    def _B_setup():
        B, S, D, F = 1, 1, 512, 1376
        return {
            "x": _w((lambda *s: _rng.normal(s) * 0.05)(B, S, D)),
            "w_gate": _w((lambda *s: _rng.normal(s) * 0.1)(D, F)),
            "w_up": _w((lambda *s: _rng.normal(s) * 0.1)(D, F)),
            "w_down": _w((lambda *s: _rng.normal(s) * 0.1)(F, D)),
        }
    _B_in = _B_setup()

    return {
        "A_x": _A_in["x"],
        "A_k_cache": _A_in["k_cache"],
        "A_v_cache": _A_in["v_cache"],
        "A_wq": _A_in["wq"],
        "A_wo": _A_in["wo"],
        "B_x": _B_in["x"],
        "B_w_gate": _B_in["w_gate"],
        "B_w_up": _B_in["w_up"],
        "B_w_down": _B_in["w_down"],
        "gate_w": _w((lambda *s: _rng.normal(s) * 0.05)(512) * 16.0),
    }

def reference(A_x, A_k_cache, A_v_cache, A_wq, A_wo, B_x, B_w_gate, B_w_up, B_w_down, gate_w):
    def _A_ref(x, k_cache, v_cache, wq, wo):
        B, Sq, D = x.shape
        Hq, Dh = 32, 128
        Hkv, Sk = k_cache.shape[1], k_cache.shape[2]
        W = min(4096, max(256, Sk // 4))
        rep = Hq // Hkv
        q = (lambda x, *d: x.transpose(*d))((x @ wq).reshape(B, Sq, Hq, Dh), 0, 2, 1, 3)
        k = jnp.repeat(k_cache[:, :, Sk - W:, :], rep, axis=1)
        v = jnp.repeat(v_cache[:, :, Sk - W:, :], rep, axis=1)
        scores = jnp.einsum("bhqd,bhkd->bhqk", q, k) * (Dh ** -0.5)
        p = _softmax(scores, axis=-1)
        o = jnp.einsum("bhqk,bhkd->bhqd", p, v)
        return (lambda x, *d: x.transpose(*d))(o, 0, 2, 1, 3).reshape(B, Sq, Hq * Dh) @ wo

    def _B_ref(x, w_gate, w_up, w_down):
        g = _silu(x @ w_gate)
        u = x @ w_up
        return (g * u) @ w_down

    x = A_x
    g = _sigmoid((x * gate_w).sum(-1, keepdims=True))
    a = _A_ref(x, A_k_cache, A_v_cache, A_wq, A_wo)
    b = _B_ref(x, B_w_gate, B_w_up, B_w_down)
    return g * a + (1 - g) * b
```

```python
import jax
import jax.numpy as jnp
from jax import lax
import jax.experimental.pallas as pl
import jax.experimental.pallas.tpu as pltpu

_NN = (((1,), (0,)), ((), ()))
_NT = (((1,), (1,)), ((), ()))

_HQ, _DH = 32, 128
_M = 8
_K_CHUNKS = (16, 16)
_V_CHUNKS = (16, 8, 8)
_WO_CHUNKS = (16, 8, 4, 2, 1, 1)


def _chunks(sizes):
    start = 0
    for size in sizes:
        yield start, size
        start += size


@jax.jit
def pallas_gated_mix__sliding_block_cached__swiglu_ffn__decode_kernel(
    A_x: jax.Array,
    A_k_cache: jax.Array,
    A_v_cache: jax.Array,
    A_wq: jax.Array,
    A_wo: jax.Array,
    B_x: jax.Array,
    B_w_gate: jax.Array,
    B_w_up: jax.Array,
    B_w_down: jax.Array,
    gate_w: jax.Array,
):
    del B_x
    D = A_x.shape[-1]
    F = B_w_down.shape[0]
    n_kv, Sk = A_k_cache.shape[1], A_k_cache.shape[2]
    assert A_x.shape == (1, 1, D) and n_kv == _HQ
    W = min(4096, max(256, Sk // 4))
    scale = _DH ** -0.5
    dt = A_x.dtype
    f32 = jnp.float32

    def kernel_function(x_hbm, k_hbm, v_hbm, wq_hbm, wo_hbm, wg_hbm, wu_hbm, wd_hbm,
                        gw_hbm, o_ref,
                        k_buf, v_buf, wq_buf, wo_buf, wg_buf, wu_buf, wd_buf,
                        x_buf, gw_buf, q_s, p_s, l_s, o_s, sems):
        n_started = [0]

        def fetch(src, dst):
            copy = pltpu.make_async_copy(src, dst, sems.at[n_started[0]])
            n_started[0] += 1
            copy.start()
            return copy

        def window(cache, start, size):
            return cache.at[0, pl.ds(start, size), pl.ds(Sk - W, W), :]

        wq_copy = fetch(wq_hbm, wq_buf)
        x_copy = fetch(x_hbm, x_buf)
        gw_copy = fetch(gw_hbm, gw_buf)
        k_copies = [fetch(window(k_hbm, a, n), k_buf.at[pl.ds(a, n)])
                    for a, n in _chunks(_K_CHUNKS)]
        v_copies = [fetch(window(v_hbm, a, n), v_buf.at[pl.ds(a, n)])
                    for a, n in _chunks(_V_CHUNKS)]
        wg_copy = fetch(wg_hbm, wg_buf)
        wu_copy = fetch(wu_hbm, wu_buf)
        wd_copy = fetch(wd_hbm, wd_buf)
        wo_copies = [fetch(wo_hbm.at[pl.ds(a * _DH, n * _DH)],
                           wo_buf.at[pl.ds(a * _DH, n * _DH)])
                     for a, n in _chunks(_WO_CHUNKS)]

        x_copy.wait()
        gw_copy.wait()
        x = x_buf[0].astype(f32)
        xs = jnp.broadcast_to(x, (_M, D)).astype(dt)
        gate = jax.nn.sigmoid(
            jnp.sum(x * gw_buf[...].astype(f32).reshape(1, D), axis=-1, keepdims=True))

        wq_copy.wait()
        q = lax.dot_general(xs, wq_buf[...], _NN, preferred_element_type=f32)
        for h in range(_HQ):
            q_s[h] = q[:, h * _DH:(h + 1) * _DH]

        def scores_step(h, carry):
            s = lax.dot_general(q_s[h].astype(dt), k_buf[h], _NT,
                                preferred_element_type=f32) * scale
            p = jnp.exp(s - jnp.max(s, axis=-1, keepdims=True))
            l_s[h] = jnp.broadcast_to(jnp.sum(p, axis=-1, keepdims=True), (_M, _DH))
            p_s[h] = p
            return carry

        for (a, n), copy in zip(_chunks(_K_CHUNKS), k_copies):
            copy.wait()
            lax.fori_loop(a, a + n, scores_step, 0)

        def values_step(h, carry):
            o = lax.dot_general(p_s[h].astype(dt), v_buf[h], _NN,
                                preferred_element_type=f32)
            o_s[h] = o / l_s[h]
            return carry

        for (a, n), copy in zip(_chunks(_V_CHUNKS), v_copies):
            copy.wait()
            lax.fori_loop(a, a + n, values_step, 0)

        wg_copy.wait()
        g = lax.dot_general(xs, wg_buf[...], _NT, preferred_element_type=f32)
        wu_copy.wait()
        u = lax.dot_general(xs, wu_buf[...], _NT, preferred_element_type=f32)
        hidden = (g * jax.nn.sigmoid(g) * u).astype(dt)
        wd_copy.wait()
        ffn = lax.dot_general(hidden, wd_buf[...], _NN, preferred_element_type=f32)

        attn = jnp.zeros((_M, D), f32)
        for (a, n), copy in zip(_chunks(_WO_CHUNKS), wo_copies):
            lhs = jnp.concatenate([o_s[h] for h in range(a, a + n)], axis=-1).astype(dt)
            copy.wait()
            attn = attn + lax.dot_general(lhs, wo_buf[a * _DH:(a + n) * _DH, :], _NN,
                                          preferred_element_type=f32)

        o_ref[0] = (gate * attn[0:1] + (1.0 - gate) * ffn[0:1]).astype(o_ref.dtype)

    n_copies = 6 + len(_K_CHUNKS) + len(_V_CHUNKS) + len(_WO_CHUNKS)
    hbm = pl.BlockSpec(memory_space=pltpu.HBM)
    return pl.pallas_call(
        kernel_function,
        out_shape=jax.ShapeDtypeStruct((1, 1, D), dt),
        in_specs=[hbm] * 9,
        out_specs=pl.BlockSpec(memory_space=pltpu.VMEM),
        scratch_shapes=[
            pltpu.VMEM((_HQ, W, _DH), dt),
            pltpu.VMEM((_HQ, W, _DH), dt),
            pltpu.VMEM((D, _HQ * _DH), dt),
            pltpu.VMEM((_HQ * _DH, D), dt),
            pltpu.VMEM((F, D), dt),
            pltpu.VMEM((F, D), dt),
            pltpu.VMEM((F, D), dt),
            pltpu.VMEM((1, 1, D), dt),
            pltpu.VMEM((D,), dt),
            pltpu.VMEM((_HQ, _M, _DH), f32),
            pltpu.VMEM((_HQ, _M, W), f32),
            pltpu.VMEM((_HQ, _M, _DH), f32),
            pltpu.VMEM((_HQ, _M, _DH), f32),
            pltpu.SemaphoreType.DMA((n_copies,)),
        ],
        compiler_params=pltpu.CompilerParams(vmem_limit_bytes=110 * 1024 * 1024),
    )(A_x, A_k_cache, A_v_cache, A_wq, A_wo, B_w_gate.T, B_w_up.T, B_w_down, gate_w)
```

```python
import jax
import jax.numpy as jnp
from jax import lax
import jax.experimental.pallas as pl
import jax.experimental.pallas.tpu as pltpu

_NN = (((1,), (0,)), ((), ()))
_NT = (((1,), (1,)), ((), ()))

_HQ, _DH = 32, 128
_SUBLANES = 8

_V_CHUNKS = (16, 8, 8)
_WO_CHUNKS = (8, 8, 4, 4, 2, 2, 1, 1, 1)
_WO_LAST_HEAD_CHUNKS = (64, 48, 16)


def _spans(sizes):
    spans, start = [], 0
    for size in sizes:
        spans.append((start, size))
        start += size
    return spans


@jax.jit
def pallas_gated_mix__sliding_block_cached__swiglu_ffn__decode_kernel(
    A_x: jax.Array,
    A_k_cache: jax.Array,
    A_v_cache: jax.Array,
    A_wq: jax.Array,
    A_wo: jax.Array,
    B_x: jax.Array,
    B_w_gate: jax.Array,
    B_w_up: jax.Array,
    B_w_down: jax.Array,
    gate_w: jax.Array,
):
    del B_x
    D = A_x.shape[-1]
    F = B_w_down.shape[0]
    Sk = A_k_cache.shape[2]
    assert A_x.shape == (1, 1, D) and D % _DH == 0
    assert A_k_cache.shape == A_v_cache.shape == (1, _HQ, Sk, _DH)
    W = min(4096, max(256, Sk // 4))
    scale = _DH ** -0.5
    dt = A_x.dtype
    f32 = jnp.float32

    v_spans = _spans(_V_CHUNKS)
    wo_spans = _spans(_WO_CHUNKS)
    last_spans = _spans(_WO_LAST_HEAD_CHUNKS)
    last_row0 = (_HQ - 1) * _DH
    n_copies = 7 + len(v_spans) + len(wo_spans) + len(last_spans)

    def kernel_function(x_hbm, k_hbm, v_hbm, wq_hbm, wo_hbm, wg_hbm, wu_hbm, wd_hbm,
                        gw_hbm, o_ref,
                        k_buf, v_buf, wq_buf, wo_buf, wg_buf, wu_buf, wd_buf,
                        x_buf, gw_buf, q_s, p_s, l_s, o_s):

        def body(sems):
            started = []

            def fetch(src, dst):
                copy = pltpu.make_async_copy(src, dst, sems.at[len(started)])
                copy.start()
                started.append(copy)
                return copy

            def window(cache, head0, n_heads):
                return cache.at[0, pl.ds(head0, n_heads), pl.ds(Sk - W, W), :]

            def fetch_wo(row0, n_rows):
                rows = pl.ds(row0, n_rows)
                return fetch(wo_hbm.at[rows], wo_buf.at[rows])

            wq_copy = fetch(wq_hbm, wq_buf)
            x_copy = fetch(x_hbm, x_buf)
            gw_copy = fetch(gw_hbm, gw_buf)
            k_copy = fetch(window(k_hbm, 0, _HQ), k_buf)
            v_copies = [fetch(window(v_hbm, a, n), v_buf.at[pl.ds(a, n)])
                        for a, n in v_spans]
            wg_copy = fetch(wg_hbm, wg_buf)
            wu_copy = fetch(wu_hbm, wu_buf)
            wd_copy = fetch(wd_hbm, wd_buf)
            wo_copies = [fetch_wo(a * _DH, n * _DH) for a, n in wo_spans]
            last_copies = [fetch_wo(last_row0 + a, n) for a, n in last_spans]

            x_copy.wait()
            gw_copy.wait()
            x = x_buf[0].astype(f32)
            xs = jnp.broadcast_to(x, (_SUBLANES, D)).astype(dt)
            gate = jax.nn.sigmoid(jnp.sum(
                x * gw_buf[...].astype(f32).reshape(1, D), axis=-1, keepdims=True))

            wq_copy.wait()
            q = lax.dot_general(xs, wq_buf[...], _NN, preferred_element_type=f32)
            for h in range(_HQ):
                q_s[h] = q[:, h * _DH:(h + 1) * _DH]

            def scores_step(h, carry):
                s = lax.dot_general(q_s[h].astype(dt), k_buf[h], _NT,
                                    preferred_element_type=f32) * scale
                p = jnp.exp(s - jnp.max(s, axis=-1, keepdims=True))
                l_s[h] = jnp.broadcast_to(jnp.sum(p, axis=-1, keepdims=True),
                                          (_SUBLANES, _DH))
                p_s[h] = p
                return carry

            k_copy.wait()
            lax.fori_loop(0, _HQ, scores_step, 0)

            def values_step(h, carry):
                o = lax.dot_general(p_s[h].astype(dt), v_buf[h], _NN,
                                    preferred_element_type=f32)
                o_s[h] = o / l_s[h]
                return carry

            for (a, n), copy in zip(v_spans, v_copies):
                copy.wait()
                lax.fori_loop(a, a + n, values_step, 0)

            wg_copy.wait()
            g = lax.dot_general(xs, wg_buf[...], _NT, preferred_element_type=f32)
            wu_copy.wait()
            u = lax.dot_general(xs, wu_buf[...], _NT, preferred_element_type=f32)
            hidden = (g * jax.nn.sigmoid(g) * u).astype(dt)
            wd_copy.wait()
            ffn = lax.dot_general(hidden, wd_buf[...], _NN, preferred_element_type=f32)

            o_last = o_s[_HQ - 1].astype(dt).astype(f32)
            o_last = jnp.broadcast_to(o_last[0:1], (_DH, _DH)).T

            attn = jnp.zeros((_SUBLANES, D), f32)
            for (a, n), copy in zip(wo_spans, wo_copies):
                lhs = jnp.concatenate([o_s[h] for h in range(a, a + n)], axis=-1)
                lhs = lhs.astype(dt)
                copy.wait()
                attn = attn + lax.dot_general(lhs, wo_buf[a * _DH:(a + n) * _DH, :],
                                              _NN, preferred_element_type=f32)
            mixed = gate * attn[0:1] + (1.0 - gate) * ffn[0:1]

            o_last = o_last * gate
            partial = jnp.zeros((_SUBLANES, D), f32)
            for (a, n), copy in zip(last_spans, last_copies):
                copy.wait()
                w = wo_buf[last_row0 + a:last_row0 + a + n, :].astype(f32)
                for r in range(0, n, _SUBLANES):
                    coeff = o_last[a + r:a + r + _SUBLANES]
                    coeff = jnp.concatenate([coeff] * (D // _DH), axis=1)
                    partial = partial + w[r:r + _SUBLANES] * coeff
            out = mixed + jnp.sum(partial, axis=0, keepdims=True)
            o_ref[0] = out.astype(o_ref.dtype)

        pl.run_scoped(body, pltpu.SemaphoreType.DMA((n_copies,)))

    return pl.pallas_call(
        kernel_function,
        out_shape=jax.ShapeDtypeStruct((1, 1, D), dt),
        in_specs=[pl.BlockSpec(memory_space=pltpu.HBM)] * 9,
        out_specs=pl.BlockSpec(memory_space=pltpu.VMEM),
        scratch_shapes=[
            pltpu.VMEM((_HQ, W, _DH), dt),
            pltpu.VMEM((_HQ, W, _DH), dt),
            pltpu.VMEM((D, _HQ * _DH), dt),
            pltpu.VMEM((_HQ * _DH, D), dt),
            pltpu.VMEM((F, D), dt),
            pltpu.VMEM((F, D), dt),
            pltpu.VMEM((F, D), dt),
            pltpu.VMEM((1, 1, D), dt),
            pltpu.VMEM((D,), dt),
            pltpu.VMEM((_HQ, _SUBLANES, _DH), f32),
            pltpu.VMEM((_HQ, _SUBLANES, W), f32),
            pltpu.VMEM((_HQ, _SUBLANES, _DH), f32),
            pltpu.VMEM((_HQ, _SUBLANES, _DH), f32),
        ],
        compiler_params=pltpu.CompilerParams(vmem_limit_bytes=100 * 1024 * 1024),
    )(A_x, A_k_cache, A_v_cache, A_wq, A_wo, B_w_gate.T, B_w_up.T, B_w_down, gate_w)
```
